```python
import jax
import jax.numpy as jnp

def _softmax(x, axis=-1):
    return jax.nn.softmax(x, axis=axis)
def _gelu(x):
    return jax.nn.gelu(x, approximate=True)
def _silu(x):
    return jax.nn.silu(x)
def _sigmoid(x):
    return jax.nn.sigmoid(x)
def _layernorm(x, axis=-1, eps=1e-5):
    m = jnp.mean(x, axis=axis, keepdims=True)
    v = jnp.var(x, axis=axis, keepdims=True)
    return (x - m) / jnp.sqrt(v + eps)
def _scatter_add(tgt, idx, src, axis=0):
    return tgt.at[idx].add(src)
def _segment_sum(src, seg, n):
    return jax.ops.segment_sum(src, seg, n)
class _Rng:
    def __init__(self, key):
        self._k = key
    def _next(self):
        self._k, sub = jax.random.split(self._k)
        return sub
    def normal(self, shape):
        return jax.random.normal(self._next(), shape, dtype=jnp.bfloat16)
    def randint(self, lo, hi, shape):
        return jax.random.randint(self._next(), shape, lo, hi, dtype=jnp.int32)
    def uniform(self, shape, lo=0.0, hi=1.0):
        return jax.random.uniform(self._next(), shape, jnp.bfloat16, lo, hi)
    def permutation(self, n):
        return jax.random.permutation(self._next(), n)


kernel_name = 'standalone__standard_2d_1d_3d_conv__vision'

def setup_inputs():
    _rng = _Rng(jax.random.key(int.from_bytes(__import__("os").urandom(4), "little")))
    _w = (lambda a: (lambda t: t.astype(jnp.bfloat16) if jnp.issubdtype(t.dtype, jnp.floating) else t)(jnp.asarray(a)))
    H = W = 384
    C = 384
    K = 1
    return {
        "x": _w((lambda *s: _rng.normal(s) * 0.05)(1, H, W, C)),
        "w": _w((lambda *s: _rng.normal(s) * 0.05)(K, K, C, C)),
        "b": _w((lambda *s: _rng.normal(s) * 0.05)(C)),
    }

def reference(x, w, b):
    B, H, W, Cin = x.shape
    K = w.shape[0]
    pl = (K - 1) // 2
    pr = K // 2
    xp = jnp.pad(x, ((0, 0), (pl, pr), (pl, pr), (0, 0)))
    out = sum(
        jnp.einsum('bhwc,cd->bhwd', xp[:, i:i+H, j:j+W, :], w[i, j])
        for i in range(K) for j in range(K)
    )
    return out + b[None, None, None, :]
```

```python
import jax
import jax.numpy as jnp
from jax import lax
import jax.experimental.pallas as pl
import jax.experimental.pallas.tpu as pltpu

SUB, LANE = 8, 128
PANELS = 3

REGIONS = 8
HEAD_REGIONS = 4
PAIRS_PER_STEP = 64
READ_TAIL = 192
WRITE_STRIDE, WRITE_PIECE, WRITE_SHIFT = 256, 8, 4


def _tiles(ref, start, count):
    return ref.at[pl.ds(start * SUB, count * SUB)]


def _strided_pieces(lo, hi):
    assert (hi - lo) % WRITE_STRIDE == 0
    cuts = sorted({0, WRITE_STRIDE, *range(WRITE_SHIFT, WRITE_STRIDE, WRITE_PIECE)})
    return [(lo, (hi - lo) // WRITE_STRIDE, a, b - a) for a, b in zip(cuts, cuts[1:])]


def _strided_view(ref, lo, strides, offset, size):
    rows = WRITE_STRIDE * SUB
    view = _tiles(ref, lo, strides * WRITE_STRIDE).reshape(strides, rows, LANE)
    return view.at[:, pl.ds(offset * SUB, size * SUB)]


def _matmul_in_place(buf, w_ref, bias, row, pairs):
    rows = pl.ds(row, pairs * 2 * PANELS * SUB)
    v = pltpu.bitcast(buf[rows, :], jnp.uint32).reshape(pairs, PANELS, SUB, LANE)
    v0, v1, v2 = v[:, 0], v[:, 1], v[:, 2]
    low = lax.broadcasted_iota(jnp.int32, (pairs, SUB, LANE), 1) < SUB // 2

    def panel_product(first, second, k):
        lhs = jnp.where(low, first, second).reshape(pairs * SUB, LANE)
        return jnp.dot(
            pltpu.bitcast(lhs, buf.dtype),
            w_ref[k * LANE:(k + 1) * LANE, :],
            preferred_element_type=jnp.float32,
        )

    p0 = panel_product(v0, v1, 0)
    p1 = panel_product(v2, v0, 1)
    p2 = panel_product(v1, v2, 2)
    p02 = (p0 + p2).reshape(pairs, 2, SUB, PANELS * LANE)
    p1 = p1.reshape(pairs, 2, SUB, PANELS * LANE)
    out_t = p02[:, 0] + p1[:, 1] + bias
    out_u = p02[:, 1] + p1[:, 0] + bias
    out = jnp.concatenate(
        [o[:, :, c * LANE:(c + 1) * LANE] for o in (out_t, out_u) for c in range(PANELS)],
        axis=1,
    )
    buf[rows, :] = out.reshape(pairs * 2 * PANELS * SUB, LANE).astype(buf.dtype)


def _conv_kernel(x_hbm, w_hbm, b_hbm, o_hbm, buf, w_ref, b_ref, read_sems, write_sem, param_sems):
    tiles = buf.shape[0] // SUB
    region = tiles // REGIONS
    step_tiles = 2 * PANELS * PAIRS_PER_STEP
    steps = region // step_tiles
    assert steps * step_tiles * REGIONS == tiles

    cuts = [g * region for g in range(REGIONS)] + [tiles - READ_TAIL, tiles]
    reads = [
        pltpu.make_async_copy(_tiles(x_hbm, a, b - a), _tiles(buf, a, b - a), read_sems.at[g])
        for g, (a, b) in enumerate(zip(cuts, cuts[1:]))
    ]
    for read in reads:
        read.start(priority=1)
    params = [
        pltpu.make_async_copy(w_hbm, w_ref, param_sems.at[0]),
        pltpu.make_async_copy(b_hbm, b_ref, param_sems.at[1]),
    ]
    for copy in params:
        copy.start(priority=0)
    for copy in params:
        copy.wait()
    bias = b_ref[...].astype(jnp.float32).reshape(1, PANELS * LANE)
    bias = jnp.broadcast_to(bias, (SUB, PANELS * LANE))

    def start_writes(lo, hi):
        for piece in _strided_pieces(lo, hi):
            pltpu.make_async_copy(
                _strided_view(buf, *piece), _strided_view(o_hbm, *piece), write_sem
            ).start()

    def do_region(g, carry):
        for h in range(HEAD_REGIONS):
            pl.when(g == h)(reads[h].wait)

        @pl.when(g == HEAD_REGIONS)
        def _switch_to_write_phase():
            for read in reads[HEAD_REGIONS:-1]:
                read.wait()
            start_writes(0, HEAD_REGIONS * region)
            reads[-1].wait()

        def step(i, carry):
            rows = step_tiles * SUB
            _matmul_in_place(buf, w_ref, bias, pl.multiple_of(i * rows, rows), PAIRS_PER_STEP)
            return carry

        lax.fori_loop(g * steps, (g + 1) * steps, step, None)

        for h in range(HEAD_REGIONS, REGIONS):
            pl.when(g == h)(lambda h=h: start_writes(h * region, (h + 1) * region))
        return carry

    lax.fori_loop(0, REGIONS, do_region, None)
    pltpu.make_async_copy(buf, buf, write_sem).wait()


@jax.jit
def pallas_standalone__standard_2d_1d_3d_conv__vision_kernel(
    x: jax.Array,
    w: jax.Array,
    b: jax.Array,
):
    channels = x.shape[-1]
    assert w.shape == (1, 1, channels, channels) and channels == PANELS * LANE
    row_tiles = x.size // (channels * SUB)

    x_tiles = x.reshape(row_tiles, SUB, PANELS, LANE).transpose(0, 2, 1, 3)
    x_tiles = x_tiles.reshape(row_tiles * PANELS * SUB, LANE)

    out_tiles = pl.pallas_call(
        _conv_kernel,
        in_specs=[pl.BlockSpec(memory_space=pl.ANY)] * 3,
        out_specs=pl.BlockSpec(memory_space=pl.ANY),
        out_shape=jax.ShapeDtypeStruct(x_tiles.shape, x.dtype),
        scratch_shapes=[
            pltpu.VMEM(x_tiles.shape, x.dtype),
            pltpu.VMEM((channels, channels), w.dtype),
            pltpu.VMEM((channels,), b.dtype),
            pltpu.SemaphoreType.DMA((REGIONS + 1,)),
            pltpu.SemaphoreType.DMA(()),
            pltpu.SemaphoreType.DMA((2,)),
        ],
        compiler_params=pltpu.CompilerParams(vmem_limit_bytes=126 * 1024 * 1024),
    )(x_tiles, w.reshape(channels, channels), b)

    out = out_tiles.reshape(row_tiles, PANELS, SUB, LANE).transpose(0, 2, 1, 3)
    return out.reshape(x.shape)
```

```python
import itertools
import math

import jax
import jax.numpy as jnp
from jax import lax
import jax.experimental.pallas as pl
import jax.experimental.pallas.tpu as pltpu

SUB, LANE = 8, 128
PANELS = 3
SLAB = 2 * PANELS

STRIDE = 256
STEP = 384
SUBSTEPS = 16
FRONT_GROUPS = (2, 2, 2, 2, 4, 4, 4, 4, 6, 6, 8, 8, 10, 10, 12, 12, 8)
LONG_PIECE = 32 * 1024 // (SUB * LANE * 2)
SHORT_STRIDES, SHORT_PIECE = 3, 8 * 1024 // (SUB * LANE * 2)
READ_STEPS = 81
WRITE_PIECE, WRITE_SHIFT = 8, 4


def _strided(ref, start, strides, offset, size):
    row, col = start * SUB, offset * SUB
    if not isinstance(row, int):
        row = pl.multiple_of(row, STRIDE * SUB)
    if not isinstance(col, int):
        col = pl.multiple_of(col, SUB)
    view = ref.at[pl.ds(row, strides * STRIDE * SUB)].reshape(strides, STRIDE * SUB, LANE)
    return view.at[:, pl.ds(col, size * SUB)]


def _wait_for(ref, sem):
    pltpu.make_async_copy(ref, ref, sem).wait()


def _segmented_loop(bounds, step, before=None, after=None):
    segments = len(bounds) - 1

    def at_segment(t, fn):
        for s in range(segments):
            pl.when(t == s)(lambda s=s: fn(s))

    def segment(t, carry):
        if before is not None:
            at_segment(t, before)
        lo, hi = bounds[0], bounds[1]
        for s in range(1, segments):
            lo = jnp.where(t >= s, bounds[s], lo)
            hi = jnp.where(t >= s, bounds[s + 1], hi)
        lax.fori_loop(lo, hi, lambda i, c: step(i), None)
        if after is not None:
            at_segment(t, after)
        return carry

    lax.fori_loop(0, segments, segment, None)


def _conv_slabs(x, w_ref, bias):
    slabs = x.shape[0] // (SLAB * SUB)
    v = pltpu.bitcast(x, jnp.uint32).reshape(slabs, PANELS, SUB, LANE)
    v0, v1, v2 = v[:, 0], v[:, 1], v[:, 2]
    first_half = lax.broadcasted_iota(jnp.int32, v0.shape, 1) < SUB // 2

    def panel_product(first, second, k):
        lhs = jnp.where(first_half, first, second).reshape(slabs * SUB, LANE)
        return jnp.dot(
            pltpu.bitcast(lhs, x.dtype),
            w_ref[k * LANE:(k + 1) * LANE, :],
            preferred_element_type=jnp.float32,
        )

    p0 = panel_product(v0, v1, 0)
    p1 = panel_product(v2, v0, 1)
    p2 = panel_product(v1, v2, 2)
    p02 = (p0 + p2).reshape(slabs, 2, SUB, PANELS * LANE)
    p1 = p1.reshape(slabs, 2, SUB, PANELS * LANE)
    out_t = p02[:, 0] + p1[:, 1] + bias
    out_u = p02[:, 1] + p1[:, 0] + bias
    out = jnp.concatenate(
        [o[:, :, c * LANE:(c + 1) * LANE] for o in (out_t, out_u) for c in range(PANELS)],
        axis=1,
    )
    return out.reshape(x.shape).astype(x.dtype)


def _conv_step(buf, w_ref, bias, step, substeps, after_substep=None):
    rows = STEP * SUB
    block = buf.at[pl.ds(pl.multiple_of(step * rows, rows), rows)]
    for j in range(substeps):
        part = pl.ds(j * rows // substeps, rows // substeps)
        out = _conv_slabs(block[part, :], w_ref, bias)
        block[part, :] = out
        if after_substep is not None:
            after_substep(j, out)


def _conv_kernel(
    x_hbm, w_hbm, b_hbm, o_hbm,
    front, back, w_ref, b_ref,
    group_sems, last_sem, short_sem, write_sem, param_sems,
):
    front_tiles = front.shape[0] // SUB
    back_tiles = x_hbm.shape[0] // SUB - front_tiles
    back_data = back.at[pl.ds(0, back_tiles * SUB)]
    spare = pl.ds(back_tiles * SUB, 2 * SUB)

    groups = len(FRONT_GROUPS)
    starts = (0, *itertools.accumulate(FRONT_GROUPS))
    passes = STRIDE // LONG_PIECE

    def group_view(ref, g, first_pass, num_passes):
        strides = FRONT_GROUPS[g] * STEP // STRIDE
        return _strided(
            ref, starts[g] * STEP, strides, first_pass * LONG_PIECE, num_passes * LONG_PIECE
        )

    def long_read(g, p, sem):
        return pltpu.make_async_copy(group_view(x_hbm, g, p, 1), group_view(front, g, p, 1), sem)

    last_read = long_read(groups - 1, passes - 1, last_sem)

    def shared_passes(g):
        return passes - 1 if g == groups - 1 else passes

    def start_group(g):
        lax.fori_loop(
            0,
            shared_passes(g),
            lambda p, c: long_read(g, p, group_sems.at[g]).start(priority=1),
            None,
            unroll=passes // 2,
        )
        if g == groups - 1:
            last_read.start(priority=1)

    def wait_group(g):
        _wait_for(group_view(front, g, 0, shared_passes(g)), group_sems.at[g])

    block = SHORT_STRIDES * STRIDE
    blocks = back_tiles // block
    short_reads = blocks * (STRIDE // SHORT_PIECE)
    slots = READ_STEPS * SUBSTEPS
    assert blocks * block == back_tiles and short_reads <= slots
    common = math.gcd(short_reads, slots)

    def start_short_read(slot):
        k = slot * (short_reads // common) // (slots // common)
        next_k = (slot + 1) * (short_reads // common) // (slots // common)

        @pl.when((slot < slots) & (next_k > k))
        def _():
            start, offset = k % blocks * block, k // blocks * SHORT_PIECE
            pltpu.make_async_copy(
                _strided(x_hbm, front_tiles + start, SHORT_STRIDES, offset, SHORT_PIECE),
                _strided(back, start, SHORT_STRIDES, offset, SHORT_PIECE),
                short_sem,
            ).start(priority=0)

    def start_writes(buf, base, lo, hi):
        strides = (hi - lo) // STRIDE
        assert strides * STRIDE == hi - lo

        def write(offset, size):
            pltpu.make_async_copy(
                _strided(buf, lo, strides, offset, size),
                _strided(o_hbm, base + lo, strides, offset, size),
                write_sem,
            ).start()

        whole = STRIDE // WRITE_PIECE - 1
        write(0, WRITE_SHIFT)
        lax.fori_loop(
            0, whole, lambda p, c: write(WRITE_SHIFT + p * WRITE_PIECE, WRITE_PIECE), None, unroll=8
        )
        write(WRITE_SHIFT + whole * WRITE_PIECE, WRITE_PIECE - WRITE_SHIFT)

    start_group(0)
    start_group(1)
    params = [
        pltpu.make_async_copy(w_hbm, w_ref, param_sems.at[0]),
        pltpu.make_async_copy(b_hbm, b_ref, param_sems.at[1]),
    ]
    for copy in params:
        copy.start(priority=0)
    for copy in params:
        copy.wait()
    bias = b_ref[...].astype(jnp.float32).reshape(1, PANELS * LANE)
    bias = jnp.broadcast_to(bias, (SUB, PANELS * LANE))

    early = [g for g in range(groups) if starts[g] < READ_STEPS]
    late = [g for g in range(groups) if starts[g] >= READ_STEPS]
    assert 1 <= len(late) <= 2
    first_writes = READ_STEPS * STEP // STRIDE * STRIDE

    def before_front_segment(s):
        if s in early:
            wait_group(s)
            if s + 2 < groups:
                start_group(s + 2)
        else:
            for g in late:
                wait_group(g)
            _wait_for(back_data, short_sem)
            start_writes(front, 0, 0, first_writes)
            last_read.wait()

    def front_step(i):
        def after_substep(j, out):
            back[spare, :] = out[:2 * SUB]
            start_short_read(i * SUBSTEPS + j)

        _conv_step(front, w_ref, bias, i, SUBSTEPS, after_substep)

    _segmented_loop(
        [*(starts[g] for g in early), READ_STEPS, starts[-1]],
        front_step,
        before=before_front_segment,
    )
    start_writes(front, 0, first_writes, front_tiles)

    halves = [0, blocks // 2 * block, back_tiles]
    _segmented_loop(
        [t // STEP for t in halves],
        lambda i: _conv_step(back, w_ref, bias, i, SUBSTEPS // 2),
        after=lambda s: start_writes(back, front_tiles, halves[s], halves[s + 1]),
    )
    _wait_for(o_hbm, write_sem)


@jax.jit
def pallas_standalone__standard_2d_1d_3d_conv__vision_kernel(
    x: jax.Array,
    w: jax.Array,
    b: jax.Array,
):
    channels = x.shape[-1]
    assert w.shape == (1, 1, channels, channels) and channels == PANELS * LANE
    row_tiles = x.size // (channels * SUB)
    front_rows = sum(FRONT_GROUPS) * STEP * SUB
    back_rows = row_tiles * PANELS * SUB - front_rows

    x_tiles = x.reshape(row_tiles, SUB, PANELS, LANE).transpose(0, 2, 1, 3)
    x_tiles = x_tiles.reshape(row_tiles * PANELS * SUB, LANE)

    out_tiles = pl.pallas_call(
        _conv_kernel,
        in_specs=[pl.BlockSpec(memory_space=pl.ANY)] * 3,
        out_specs=pl.BlockSpec(memory_space=pl.ANY),
        out_shape=jax.ShapeDtypeStruct(x_tiles.shape, x.dtype),
        scratch_shapes=[
            pltpu.VMEM((front_rows, LANE), x.dtype),
            pltpu.VMEM((back_rows + 2 * SUB, LANE), x.dtype),
            pltpu.VMEM((channels, channels), w.dtype),
            pltpu.VMEM((channels,), b.dtype),
            pltpu.SemaphoreType.DMA((len(FRONT_GROUPS),)),
            pltpu.SemaphoreType.DMA(()),
            pltpu.SemaphoreType.DMA(()),
            pltpu.SemaphoreType.DMA(()),
            pltpu.SemaphoreType.DMA((2,)),
        ],
        compiler_params=pltpu.CompilerParams(
            vmem_limit_bytes=126 * 1024 * 1024,
            disable_bounds_checks=True,
        ),
    )(x_tiles, w.reshape(channels, channels), b)

    out = out_tiles.reshape(row_tiles, PANELS, SUB, LANE).transpose(0, 2, 1, 3)
    return out.reshape(x.shape)
```

```python
import itertools
import math

import jax
import jax.numpy as jnp
from jax import lax
import jax.experimental.pallas as pl
import jax.experimental.pallas.tpu as pltpu

SUB, LANE = 8, 128
PANELS = 3
SLAB = 2 * PANELS * SUB

LINE = 2048
LONG_PIECE = 128
SHORT_PIECE = 32
WRITE_PIECE, WRITE_SHIFT = 64, 32

STEP = 3
SUBSTEPS = 32
FRONT_GROUPS = (1, 1, 1, 1, 1, 2, 2, 2, 2, 2, 3, 3, 4, 4, 4, 4, 5, 6, 4)
READ_STEPS = 42


def _wait_for(ref, sem):
    pltpu.make_async_copy(ref, ref, sem).wait()


def _segmented_loop(bounds, step, before=None, after=None):
    segments = len(bounds) - 1

    def at_segment(t, fn):
        for s in range(segments):
            pl.when(t == s)(lambda s=s: fn(s))

    def segment(t, carry):
        if before is not None:
            at_segment(t, before)
        lo, hi = bounds[0], bounds[1]
        for s in range(1, segments):
            lo = jnp.where(t >= s, bounds[s], lo)
            hi = jnp.where(t >= s, bounds[s + 1], hi)
        lax.fori_loop(lo, hi, lambda i, c: step(i), None)
        if after is not None:
            at_segment(t, after)
        return carry

    lax.fori_loop(0, segments, segment, None)


def _conv_slabs(x, w_ref, bias):
    slabs = x.shape[0] // SLAB
    v = pltpu.bitcast(x, jnp.uint32).reshape(slabs, PANELS, SUB, LANE)
    v0, v1, v2 = v[:, 0], v[:, 1], v[:, 2]
    first_half = lax.broadcasted_iota(jnp.int32, v0.shape, 1) < SUB // 2

    def panel_product(first, second, k):
        lhs = jnp.where(first_half, first, second).reshape(slabs * SUB, LANE)
        return jnp.dot(
            pltpu.bitcast(lhs, x.dtype),
            w_ref[k * LANE:(k + 1) * LANE, :],
            preferred_element_type=jnp.float32,
        )

    p0 = panel_product(v0, v1, 0)
    p1 = panel_product(v2, v0, 1)
    p2 = panel_product(v1, v2, 2)
    p02 = (p0 + p2).reshape(slabs, 2, SUB, PANELS * LANE)
    p1 = p1.reshape(slabs, 2, SUB, PANELS * LANE)
    out_t = p02[:, 0] + p1[:, 1] + bias
    out_u = p02[:, 1] + p1[:, 0] + bias
    out = jnp.concatenate(
        [o[:, :, c * LANE:(c + 1) * LANE] for o in (out_t, out_u) for c in range(PANELS)],
        axis=1,
    )
    return out.reshape(x.shape).astype(x.dtype)


def _conv_step(buf, w_ref, bias, step, substeps, after_substep=None):
    lines = buf.at[pl.ds(step * STEP, STEP)]
    rows = STEP * LINE // substeps
    for j in range(substeps):
        lo, hi = j * rows, (j + 1) * rows
        cuts = [lo, *range((lo // LINE + 1) * LINE, hi, LINE), hi]
        parts = [(a // LINE, pl.ds(a % LINE, b - a)) for a, b in zip(cuts, cuts[1:])]
        out = _conv_slabs(jnp.concatenate([lines[part] for part in parts]), w_ref, bias)
        for part, a, b in zip(parts, cuts, cuts[1:]):
            lines[part] = out[a - lo:b - lo]
        if after_substep is not None:
            after_substep(j, out)


def _conv_kernel(
    x_hbm, w_hbm, b_hbm, o_hbm,
    front, back, w_ref, b_ref,
    group_sems, last_sem, short_sem, write_sem, param_sems,
):
    front_lines = front.shape[0]
    back_lines = x_hbm.shape[0] - front_lines

    groups = len(FRONT_GROUPS)
    starts = (0, *itertools.accumulate(FRONT_GROUPS))
    passes = LINE // LONG_PIECE

    def group_view(ref, g, row, rows):
        return ref.at[pl.ds(starts[g] * STEP, FRONT_GROUPS[g] * STEP), pl.ds(row, rows)]

    def long_read(g, row, sem):
        return pltpu.make_async_copy(
            group_view(x_hbm, g, row, LONG_PIECE), group_view(front, g, row, LONG_PIECE), sem
        )

    last_read = long_read(groups - 1, LINE - LONG_PIECE, last_sem)

    def shared_passes(g):
        return passes - 1 if g == groups - 1 else passes

    def start_group(g):
        def start_pass(p, carry):
            row = pl.multiple_of(p * LONG_PIECE, LONG_PIECE)
            long_read(g, row, group_sems.at[g]).start(priority=1)
            return carry

        lax.fori_loop(0, shared_passes(g), start_pass, None, unroll=passes // 2)
        if g == groups - 1:
            last_read.start(priority=1)

    def wait_group(g):
        _wait_for(group_view(front, g, 0, shared_passes(g) * LONG_PIECE), group_sems.at[g])

    back_steps = back_lines // STEP
    short_reads = back_steps * (LINE // SHORT_PIECE)
    slots = READ_STEPS * SUBSTEPS
    assert back_steps * STEP == back_lines and short_reads <= slots
    common = math.gcd(short_reads, slots)

    def start_short_read(slot):
        k = slot * (short_reads // common) // (slots // common)
        next_k = (slot + 1) * (short_reads // common) // (slots // common)

        @pl.when((slot < slots) & (next_k > k))
        def _():
            line = k % back_steps * STEP
            rows = pl.ds(pl.multiple_of(k // back_steps * SHORT_PIECE, SHORT_PIECE), SHORT_PIECE)
            pltpu.make_async_copy(
                x_hbm.at[pl.ds(front_lines + line, STEP), rows],
                back.at[pl.ds(line, STEP), rows],
                short_sem,
            ).start(priority=0)

    def start_writes(buf, base, lo, hi):
        def write(row, rows):
            pltpu.make_async_copy(
                buf.at[pl.ds(lo, hi - lo), pl.ds(row, rows)],
                o_hbm.at[pl.ds(base + lo, hi - lo), pl.ds(row, rows)],
                write_sem,
            ).start()

        def write_piece(p, carry):
            write(pl.multiple_of(WRITE_SHIFT + p * WRITE_PIECE, WRITE_SHIFT), WRITE_PIECE)
            return carry

        whole = LINE // WRITE_PIECE - 1
        write(0, WRITE_SHIFT)
        lax.fori_loop(0, whole, write_piece, None, unroll=8)
        write(WRITE_SHIFT + whole * WRITE_PIECE, WRITE_PIECE - WRITE_SHIFT)

    start_group(0)
    start_group(1)
    params = [
        pltpu.make_async_copy(w_hbm, w_ref, param_sems.at[0]),
        pltpu.make_async_copy(b_hbm, b_ref, param_sems.at[1]),
    ]
    for copy in params:
        copy.start(priority=0)
    for copy in params:
        copy.wait()
    bias = b_ref[...].astype(jnp.float32).reshape(1, PANELS * LANE)
    bias = jnp.broadcast_to(bias, (SUB, PANELS * LANE))

    early = [g for g in range(groups) if starts[g] < READ_STEPS]
    late = [g for g in range(groups) if starts[g] >= READ_STEPS]
    assert 1 <= len(late) <= 2

    def before_front_segment(s):
        if s in early:
            wait_group(s)
            if s + 2 < groups:
                start_group(s + 2)
        else:
            for g in late:
                wait_group(g)
            _wait_for(back.at[pl.ds(0, back_lines)], short_sem)
            start_writes(front, 0, 0, READ_STEPS * STEP)
            last_read.wait()

    def front_step(i):
        def after_substep(j, out):
            back[back_lines, :2 * SUB] = out[:2 * SUB]
            start_short_read(i * SUBSTEPS + j)

        _conv_step(front, w_ref, bias, i, SUBSTEPS, after_substep)

    _segmented_loop(
        [*(starts[g] for g in early), READ_STEPS, starts[-1]],
        front_step,
        before=before_front_segment,
    )
    start_writes(front, 0, READ_STEPS * STEP, front_lines)

    halves = [0, back_steps // 2, back_steps]
    _segmented_loop(
        halves,
        lambda i: _conv_step(back, w_ref, bias, i, SUBSTEPS // 2),
        after=lambda s: start_writes(back, front_lines, halves[s] * STEP, halves[s + 1] * STEP),
    )
    _wait_for(o_hbm, write_sem)


@jax.jit
def pallas_standalone__standard_2d_1d_3d_conv__vision_kernel(
    x: jax.Array,
    w: jax.Array,
    b: jax.Array,
):
    channels = x.shape[-1]
    assert w.shape == (1, 1, channels, channels) and channels == PANELS * LANE
    row_tiles = x.size // (channels * SUB)
    lines = row_tiles * PANELS * SUB // LINE
    front_lines = sum(FRONT_GROUPS) * STEP

    x_tiles = x.reshape(row_tiles, SUB, PANELS, LANE).transpose(0, 2, 1, 3)
    x_tiles = x_tiles.reshape(lines, LINE, LANE)

    out_tiles = pl.pallas_call(
        _conv_kernel,
        in_specs=[pl.BlockSpec(memory_space=pl.ANY)] * 3,
        out_specs=pl.BlockSpec(memory_space=pl.ANY),
        out_shape=jax.ShapeDtypeStruct(x_tiles.shape, x.dtype),
        scratch_shapes=[
            pltpu.VMEM((front_lines, LINE, LANE), x.dtype),
            pltpu.VMEM((lines - front_lines + 1, LINE, LANE), x.dtype),
            pltpu.VMEM((channels, channels), w.dtype),
            pltpu.VMEM((channels,), b.dtype),
            pltpu.SemaphoreType.DMA((len(FRONT_GROUPS),)),
            pltpu.SemaphoreType.DMA(()),
            pltpu.SemaphoreType.DMA(()),
            pltpu.SemaphoreType.DMA(()),
            pltpu.SemaphoreType.DMA((2,)),
        ],
        compiler_params=pltpu.CompilerParams(
            vmem_limit_bytes=116 * 1024 * 1024,
            disable_bounds_checks=True,
        ),
    )(x_tiles, w.reshape(channels, channels), b)

    out = out_tiles.reshape(row_tiles, PANELS, SUB, LANE).transpose(0, 2, 1, 3)
    return out.reshape(x.shape)
```
